```python
import jax
import jax.numpy as jnp

def _softmax(x, axis=-1):
    return jax.nn.softmax(x, axis=axis)
def _gelu(x):
    return jax.nn.gelu(x, approximate=True)
def _silu(x):
    return jax.nn.silu(x)
def _sigmoid(x):
    return jax.nn.sigmoid(x)
def _layernorm(x, axis=-1, eps=1e-5):
    m = jnp.mean(x, axis=axis, keepdims=True)
    v = jnp.var(x, axis=axis, keepdims=True)
    return (x - m) / jnp.sqrt(v + eps)
def _scatter_add(tgt, idx, src, axis=0):
    return tgt.at[idx].add(src)
def _segment_sum(src, seg, n):
    return jax.ops.segment_sum(src, seg, n)
class _Rng:
    def __init__(self, key):
        self._k = key
    def _next(self):
        self._k, sub = jax.random.split(self._k)
        return sub
    def normal(self, shape):
        return jax.random.normal(self._next(), shape, dtype=jnp.bfloat16)
    def randint(self, lo, hi, shape):
        return jax.random.randint(self._next(), shape, lo, hi, dtype=jnp.int32)
    def uniform(self, shape, lo=0.0, hi=1.0):
        return jax.random.uniform(self._next(), shape, jnp.bfloat16, lo, hi)
    def permutation(self, n):
        return jax.random.permutation(self._next(), n)


kernel_name = 'interleave_layers__ssm_conv_h3__mixer_s_mlp__prompt'

def setup_inputs():
    _rng = _Rng(jax.random.key(int.from_bytes(__import__("os").urandom(4), "little")))
    _w = (lambda a: (lambda t: t.astype(jnp.bfloat16) if jnp.issubdtype(t.dtype, jnp.floating) else t)(jnp.asarray(a)))
    def _A_setup():
        B, S, D = 1, 2048, 1024
        ks = 4
        return {
            "q": _w((lambda *s: _rng.normal(s) * 0.05)(B, S, D)),
            "k": _w((lambda *s: _rng.normal(s) * 0.05)(B, S, D)),
            "v": _w((lambda *s: _rng.normal(s) * 0.05)(B, S, D)),
            "shift_k": _w((lambda *s: _rng.normal(s) * 0.05)(D, ks) * 0.5),
            "ssm_k": _w((lambda *s: _rng.normal(s) * 0.05)(D, S) * (1.0 / S ** 0.5)),
            "ssm_D": _w((lambda *s: _rng.normal(s) * 0.05)(D)),
        }
    _A_in = _A_setup()

    def _B_setup():
        B, S, D, F = 1, 2048, 1024, 3584
        return {
            "x":  _w((lambda *s: _rng.normal(s) * 0.05)(B, S, D)),
            "w1": _w((lambda *s: _rng.normal(s) * 0.05)(D, D) * (D ** -0.5)),
            "w2": _w((lambda *s: _rng.normal(s) * 0.05)(D, D) * (D ** -0.5)),
            "w3": _w((lambda *s: _rng.normal(s) * 0.05)(D, F) * (D ** -0.5)),
            "w4": _w((lambda *s: _rng.normal(s) * 0.05)(F, D) * (F ** -0.5)),
        }
    _B_in = _B_setup()

    return {
        "A_q": _A_in["q"],
        "A_k": _A_in["k"],
        "A_v": _A_in["v"],
        "A_shift_k": _A_in["shift_k"],
        "A_ssm_k": _A_in["ssm_k"],
        "A_ssm_D": _A_in["ssm_D"],
        "B_x": _B_in["x"],
        "B_w1": _B_in["w1"],
        "B_w2": _B_in["w2"],
        "B_w3": _B_in["w3"],
        "B_w4": _B_in["w4"],
    }

def reference(A_q, A_k, A_v, A_shift_k, A_ssm_k, A_ssm_D, B_x, B_w1, B_w2, B_w3, B_w4):
    def _A_ref(q, k, v, shift_k, ssm_k, ssm_D):
        B, S, D = q.shape
        ks = shift_k.shape[-1]
        k_pad = jnp.pad(k, ((0, 0), (ks - 1, 0), (0, 0)))
        k_shift = jnp.zeros_like(k)
        for t in range(ks):
            k_shift = k_shift + k_pad[:, t:t + S, :] * shift_k[:, ks - 1 - t][None, None, :]
        kv = k_shift * v
        L = 2 * S
        kv_pad = jnp.pad(kv, ((0, 0), (0, S), (0, 0)))
        kf_pad = jnp.pad(ssm_k, ((0, 0), (0, S)))
        kv_f = (lambda x, axes=(-2,-1): jnp.fft.rfft2(x.astype(jnp.float32), axes=axes))(kv_pad[:, None, :, :], axes=(1, 2))
        kf_f = (lambda x, axes=(-2,-1): jnp.fft.rfft2(x.astype(jnp.float32), axes=axes))(kf_pad[:, None, :], axes=(1, 2))
        kf_f = (lambda x, *d: x.transpose(*d))(kf_f, 1, 2, 0)
        y_f = kv_f * kf_f[None, :, :, :]
        y = (lambda x, s, axes=(-2,-1): jnp.fft.irfft2(x, s=s, axes=axes).astype(jnp.bfloat16))(y_f, (1, L), axes=(1, 2))[:, 0, :S, :]
        y = y + kv * ssm_D[None, None, :]
        return q * y

    def _B_ref(x, w1, w2, w3, w4):
        B, S, D = x.shape
        h = _gelu(_layernorm(x, axis=-1) @ w1)
        c = D // 4
        g0 = jnp.pad(h[:, :, 0*c:1*c], ((0, 0), (1, 0), (0, 0)))[:, :S, :]
        g1 = jnp.pad(h[:, :, 1*c:2*c], ((0, 0), (0, 1), (0, 0)))[:, 1:, :]
        g2 = jnp.pad(h[:, :, 2*c:3*c], ((0, 0), (2, 0), (0, 0)))[:, :S, :]
        g3 = jnp.pad(h[:, :, 3*c:   ], ((0, 0), (0, 2), (0, 0)))[:, 2:, :]
        hs = jnp.concatenate([g0, g1, g2, g3], axis=-1) @ w2
        x1 = x + hs
        h2 = _gelu(_layernorm(x1, axis=-1) @ w3) @ w4
        return x1 + h2

    x = A_q
    x = x + _A_ref(_layernorm(x, axis=-1), A_k, A_v, A_shift_k, A_ssm_k, A_ssm_D)
    x = x + _B_ref(_layernorm(x, axis=-1), B_w1, B_w2, B_w3, B_w4)
    x = x + _A_ref(_layernorm(x, axis=-1), A_k, A_v, A_shift_k, A_ssm_k, A_ssm_D)
    x = x + _B_ref(_layernorm(x, axis=-1), B_w1, B_w2, B_w3, B_w4)
    return x
```

```python
import numpy as np
import jax
import jax.numpy as jnp
from jax import lax
import jax.experimental.pallas as pl
import jax.experimental.pallas.tpu as pltpu

S, D, F = 2048, 1024, 3584
TB = 128
NB = S // TB
CC = 256
NC = D // CC
TM = 256
NT = S // TM
FC = 256
RS = 128
EPS = 1e-5
MODE = 0
U = 1
f32, bf16 = jnp.float32, jnp.bfloat16


def _dft_mats():
    t = np.arange(TB)
    ang = 2 * np.pi * np.outer(t + 0.5, t) / (2 * TB)
    fwd = np.concatenate([np.cos(ang), -np.sin(ang)], 0)
    return fwd.astype(np.float32), (fwd.T / TB).astype(np.float32)


def _ln(x):
    m = jnp.mean(x, axis=-1, keepdims=True)
    c = x - m
    v = jnp.mean(c * c, axis=-1, keepdims=True)
    return c * lax.rsqrt(v + EPS)


def _gelu(x):
    c0 = float(np.sqrt(2 / np.pi))
    u = x * (x * x * (0.044715 * c0) + c0)
    hx = 0.5 * x
    return hx * jnp.tanh(u) + hx


def _dot(a, b):
    return jnp.dot(a, b, preferred_element_type=f32)


def _kernel(q_h, k_h, v_h, sk_ref, ssm_h, sd_ref, w1_h, w2_h, w3_h, w4_h,
            fw_ref, iv_ref, out_h,
            qb, w1, w2, w3, w4, yb, sem_in, sem_w, sem_o):
    wcopies = [pltpu.make_async_copy(a, b, sem_w.at[i]) for i, (a, b) in
               enumerate(((q_h, qb), (w1_h, w1), (w2_h, w2), (w3_h, w3), (w4_h, w4)))]

    def conv(kb, vb, sb, kvb, XS, KS, ZS):
        cps = []
        for c in range(NC):
            cs = pl.ds(c * CC, CC)
            cps.append([
                pltpu.make_async_copy(k_h.at[:, cs], kb.at[c], sem_in.at[3 * c]),
                pltpu.make_async_copy(v_h.at[:, cs], vb.at[c], sem_in.at[3 * c + 1]),
                pltpu.make_async_copy(ssm_h.at[cs, :], sb.at[c], sem_in.at[3 * c + 2]),
            ])
        later = [wcopies[:1], wcopies[1:3], wcopies[3:4], wcopies[4:]]
        for cp in cps[0]:
            cp.start()

        for c in range(NC):
            cps[c][0].wait()
            if c + 1 < NC:
                for cp in cps[c + 1]:
                    cp.start()
            for cp in later[c]:
                cp.start()
            cps[c][1].wait()
            taps = [sk_ref[j:j + 1, c * CC:(c + 1) * CC] for j in range(4)]
            fw = fw_ref[...]

            for j in range(NB):
                r0 = j * TB
                if j == 0:
                    kw = jnp.concatenate(
                        [jnp.zeros((16, CC), f32), kb[c, 0:TB, :].astype(f32)], 0)
                else:
                    kw = kb[c, r0 - 16:r0 + TB, :].astype(f32)
                ks = kw[16:] * taps[0]
                for t in range(1, 4):
                    ks = ks + pltpu.roll(kw, t, 0)[16:] * taps[t]
                kv = ks * vb[c, r0:r0 + TB, :].astype(f32)
                kvb[r0:r0 + TB, :] = kv
                X = _dot(fw, kv.astype(bf16))
                XS[j, 0:2 * TB, :] = X
                XS[j, 2 * TB:, :] = X[:TB] + X[TB:]

            sg = 1.0 - 2.0 * (lax.broadcasted_iota(jnp.int32, (TB, CC), 0) & 1).astype(f32)
            prev = None
            cps[c][2].wait()
            for m in range(NB):
                K = lax.dot_general(fw, sb[c, :, m * TB:(m + 1) * TB],
                                    (((1,), (1,)), ((), ())), preferred_element_type=f32)
                kr, ki = K[:TB], K[TB:]
                if prev is not None:
                    kr = kr - sg * prev[TB:]
                    ki = ki + sg * prev[:TB]
                prev = K
                KS[m, 0:TB, :] = kr + ki
                KS[m, TB:2 * TB, :] = ki - kr
                KS[m, 2 * TB:, :] = kr

            def pos(p, _):
                r = pl.multiple_of(p * 8, 8)
                for l in range(CC // 128):
                    ls = pl.ds(l * 128, 128)
                    ld = lambda ref, b, comp: ref[b, pl.ds(r + comp * TB, 8), ls]
                    for i0 in range(0, NB, 4):
                        acc = [[None] * 3 for _ in range(4)]
                        for j in range(i0 + 4):
                            a, b, ab = ld(XS, j, 0), ld(XS, j, 1), ld(XS, j, 2)
                            for ii in range(4):
                                m = i0 + ii - j
                                if m < 0:
                                    continue
                                t = (b * ld(KS, m, 0), a * ld(KS, m, 1), ab * ld(KS, m, 2))
                                acc[ii] = [u if o is None else o + u
                                           for o, u in zip(acc[ii], t)]
                        for ii in range(4):
                            ZS[i0 + ii, pl.ds(r, 8), ls] = acc[ii][2] - acc[ii][0]
                            ZS[i0 + ii, pl.ds(r + TB, 8), ls] = acc[ii][2] + acc[ii][1]
                return 0
            lax.fori_loop(0, TB // 8, pos, 0)

            iv = iv_ref[...]
            sd = sd_ref[:, c * CC:(c + 1) * CC]
            for i in range(NB):
                r0 = i * TB
                y = _dot(iv, ZS[i].astype(bf16)) + kvb[r0:r0 + TB, :] * sd
                yb[r0:r0 + TB, c * CC:(c + 1) * CC] = y

    pl.run_scoped(
        conv,
        pltpu.VMEM((NC, S, CC), bf16), pltpu.VMEM((NC, S, CC), bf16),
        pltpu.VMEM((NC, CC, S), bf16), pltpu.VMEM((S, CC), f32),
        pltpu.VMEM((NB, 3 * TB, CC), f32), pltpu.VMEM((NB, 3 * TB, CC), f32),
        pltpu.VMEM((NB, 2 * TB, CC), f32))

    def mixer(xa, xn, H, ob, nb):
        G = D // 4
        for l in range(2):
            H[l, 0:8, :] = jnp.zeros((8, D), f32)
            H[l, 8 + S:, :] = jnp.zeros((8, D), f32)

        def rows(t):
            return pl.ds(t * TM if isinstance(t, int) else pl.multiple_of(t * TM, TM), TM)

        def pre(src, t, l):
            n2 = []
            for u in range(TM // RS):
                rs = pl.ds(rows(t).start + u * RS, RS)
                x = src[rs, :].astype(f32)
                x = x + _ln(x) * yb[rs, :]
                n = _ln(x)
                xa[rs, :] = x
                xn[rs, :] = n
                n2.append(_ln(n).astype(bf16))
                yield
            H[l, pl.ds(rows(t).start + 8, TM), :] = _gelu(
                _dot(jnp.concatenate(n2, 0), w1[...]))

        def mix(t, l):
            parts = []
            for g, sh in enumerate((1, -1, 2, -2)):
                w = H[l, pl.ds(rows(t).start, TM + 16), g * G:(g + 1) * G]
                parts.append(pltpu.roll(w, sh % (TM + 16), 0)[8:8 + TM].astype(bf16))
                yield
            x1 = xn[rows(t), :] + _dot(jnp.concatenate(parts, 1), w2[...])
            yield
            for u in range(TM // RS):
                rs = pl.ds(rows(t).start + u * RS, RS)
                xu = x1[u * RS:(u + 1) * RS]
                nb[t % 2, u * RS:(u + 1) * RS, :] = _ln(xu).astype(bf16)
                xa[rs, :] = xa[rs, :] + xu
                yield

        def mlp(t, l):
            n1 = nb[t % 2]
            acc = xa[rows(t), :]
            for fc in range(F // FC):
                g = _gelu(_dot(n1, w3[:, fc * FC:(fc + 1) * FC])).astype(bf16)
                yield
                acc = acc + _dot(g, w4[fc * FC:(fc + 1) * FC, :])
                yield
            if l == 0:
                xa[rows(t), :] = acc
            else:
                ob[rows(t), :] = acc.astype(bf16)
                ocp(t).start()

        def ocp(t):
            return pltpu.make_async_copy(ob.at[rows(t)], out_h.at[rows(t)], sem_o.at[t])

        def chain(*gs):
            for g in gs:
                yield from g
                yield

        def weave(a, b):
            for _ in a:
                next(b, None)
            for _ in b:
                pass

        wcopies[0].wait()
        wcopies[1].wait()

        def s0(t, _):
            weave(pre(qb, t, 0), iter(()))
            return 0
        lax.fori_loop(0, 2, s0, 0)
        for cp in wcopies[2:]:
            cp.wait()
        weave(mix(0, 0), iter(()))
        weave(mlp(0, 0), chain(pre(qb, 2, 0), mix(1, 0)))

        def s1(t, _):
            weave(mlp(t, 0), chain(pre(qb, t + 2, 0), mix(t + 1, 0), pre(xa, t - 1, 1)))
            return 0
        lax.fori_loop(1, NT - 2, s1, 0)
        weave(mlp(NT - 2, 0), chain(mix(NT - 1, 0), pre(xa, NT - 3, 1)))
        weave(mlp(NT - 1, 0), chain(pre(xa, NT - 2, 1), mix(0, 1)))
        weave(mlp(0, 1), chain(pre(xa, NT - 1, 1), mix(1, 1)))

        def s2(t, _):
            weave(mlp(t, 1), mix(t + 1, 1))
            return 0
        lax.fori_loop(1, NT - 1, s2, 0)
        weave(mlp(NT - 1, 1), iter(()))
        for t in range(NT):
            ocp(t).wait()

    if MODE == 1:
        def dbg(ob):
            for cp in wcopies:
                cp.wait()
            ob[...] = (yb[...] * 1e5).astype(bf16)
            cp = pltpu.make_async_copy(ob, out_h, sem_o.at[0])
            cp.start()
            cp.wait()
        pl.run_scoped(dbg, pltpu.VMEM((S, D), bf16))
        return
    pl.run_scoped(mixer, pltpu.VMEM((S, D), f32), pltpu.VMEM((S, D), f32),
                  pltpu.VMEM((2, S + 16, D), f32), pltpu.VMEM((S, D), bf16), pltpu.VMEM((2, TM, D), bf16))


@jax.jit
def pallas_interleave_layers__ssm_conv_h3__mixer_s_mlp__prompt_kernel(
    A_q, A_k, A_v, A_shift_k, A_ssm_k, A_ssm_D, B_x, B_w1, B_w2, B_w3, B_w4,
):
    del B_x
    fw, iv = _dft_mats()
    hbm = pl.BlockSpec(memory_space=pl.ANY)
    vm = pl.BlockSpec(memory_space=pltpu.VMEM)
    out = pl.pallas_call(
        _kernel,
        out_shape=jax.ShapeDtypeStruct((S, D), bf16),
        in_specs=[hbm, hbm, hbm, vm, hbm, vm, hbm, hbm, hbm, hbm, vm, vm],
        out_specs=hbm,
        scratch_shapes=[
            pltpu.VMEM((S, D), bf16), pltpu.VMEM((D, D), bf16), pltpu.VMEM((D, D), bf16),
            pltpu.VMEM((D, F), bf16), pltpu.VMEM((F, D), bf16), pltpu.VMEM((S, D), f32),
            pltpu.SemaphoreType.DMA((3 * NC,)), pltpu.SemaphoreType.DMA((5,)),
            pltpu.SemaphoreType.DMA((NT,)),
        ],
        compiler_params=pltpu.CompilerParams(vmem_limit_bytes=120 * 1024 * 1024),
    )(A_q.reshape(S, D), A_k.reshape(S, D), A_v.reshape(S, D),
      A_shift_k.T.astype(f32), A_ssm_k, A_ssm_D.reshape(1, D).astype(f32),
      B_w1, B_w2, B_w3, B_w4, jnp.asarray(fw, bf16), jnp.asarray(iv, bf16))
    return out.reshape(1, S, D)
```

```python
import numpy as np
import jax
import jax.numpy as jnp
from jax import lax
import jax.experimental.pallas as pl
import jax.experimental.pallas.tpu as pltpu

S, D, F = 2048, 1024, 3584
TB = 128
NB = S // TB
CC = 256
NC = D // CC
TM = 256
NT = S // TM
FC = 256
RS = 256
EPS = 1e-5
PU = 1
SK = 3
f32, bf16 = jnp.float32, jnp.bfloat16


def _dft_mats():
    t = np.arange(TB)
    ang = 2 * np.pi * np.outer(t + 0.5, t) / (2 * TB)
    fwd = np.concatenate([np.cos(ang), -np.sin(ang)], 0)
    return fwd.astype(np.float32), (fwd.T / TB).astype(np.float32)


def _ln(x):
    m = jnp.mean(x, axis=-1, keepdims=True)
    c = x - m
    v = jnp.mean(c * c, axis=-1, keepdims=True)
    return c * lax.rsqrt(v + EPS)


def _gelu(x):
    c0 = float(np.sqrt(2 / np.pi))
    u = x * (x * x * (0.044715 * c0) + c0)
    hx = 0.5 * x
    return hx * jnp.tanh(u) + hx


def _dot(a, b):
    return jnp.dot(a, b, preferred_element_type=f32)


def _kernel(q_h, k_h, v_h, sk_ref, ssm_h, sd_ref, w1_h, w2_h, w3_h, w4_h,
            fw_ref, iv_ref, out_h,
            qb, w1, w2, w3, w4, yb, XS, KS, ZS, sem_in, sem_w, sem_o):
    FH = F // 2
    wcopies = [pltpu.make_async_copy(a, b, sem_w.at[i]) for i, (a, b) in enumerate((
        (q_h, qb), (w1_h, w1), (w2_h, w2),
        (w3_h.at[:, :FH], w3.at[:, :FH]), (w4_h.at[:FH], w4.at[:FH]),
        (w3_h.at[:, FH:], w3.at[:, FH:]), (w4_h.at[FH:], w4.at[FH:])))]

    def spec(zc, r, l, i0):
        ls = pl.ds(l * 128, 128)
        ld = lambda ref, b, comp: ref[b, pl.ds(r + comp * TB, 8), ls]
        acc = [[None] * 3 for _ in range(4)]
        for j in range(i0 + 4):
            a, b, ab = ld(XS, j, 0), ld(XS, j, 1), ld(XS, j, 2)
            for ii in range(4):
                m = i0 + ii - j
                if m >= 0:
                    t = (b * ld(KS, m, 0), a * ld(KS, m, 1), ab * ld(KS, m, 2))
                    acc[ii] = [u if o is None else o + u for o, u in zip(acc[ii], t)]
        for ii in range(4):
            ZS[zc, ii, pl.ds(r, 8), ls] = acc[ii][2] - acc[ii][0]
            ZS[zc, ii, pl.ds(r + TB, 8), ls] = acc[ii][2] + acc[ii][1]

    def inv(c, zc, i0):
        for ii in range(4):
            rs = pl.ds((i0 + ii) * TB, TB)
            yb[c, rs, :] = yb[c, rs, :] + _dot(iv_ref[...], ZS[zc, ii].astype(bf16))

    def conv(kb, vb, sb):
        cps = []
        for c in range(NC):
            cs = pl.ds(c * CC, CC)
            cps.append([
                pltpu.make_async_copy(k_h.at[:, cs], kb.at[c], sem_in.at[3 * c]),
                pltpu.make_async_copy(v_h.at[:, cs], vb.at[c], sem_in.at[3 * c + 1]),
                pltpu.make_async_copy(ssm_h.at[cs, :], sb.at[c], sem_in.at[3 * c + 2]),
            ])
        later = [wcopies[:1], wcopies[1:3], wcopies[3:5], wcopies[5:]]
        for cp in cps[0]:
            cp.start()

        for c in range(NC):
            cps[c][0].wait()
            if c + 1 < NC:
                for cp in cps[c + 1]:
                    cp.start()
            for cp in later[c]:
                cp.start()
            cps[c][1].wait()
            taps = [sk_ref[j:j + 1, c * CC:(c + 1) * CC] for j in range(4)]
            sd = sd_ref[:, c * CC:(c + 1) * CC]
            fw = fw_ref[...]
            for j in range(NB):
                r0 = j * TB
                if j == 0:
                    kw = jnp.concatenate(
                        [jnp.zeros((16, CC), f32), kb[c, 0:TB, :].astype(f32)], 0)
                else:
                    kw = kb[c, r0 - 16:r0 + TB, :].astype(f32)
                kw = kw[8:]
                ks = kw[8:] * taps[0]
                for t in range(1, 4):
                    ks = ks + pltpu.roll(kw, t, 0)[8:] * taps[t]
                kv = ks * vb[c, r0:r0 + TB, :].astype(f32)
                yb[c, r0:r0 + TB, :] = kv * sd
                X = _dot(fw, kv.astype(bf16))
                XS[j, :2 * TB, :] = X
                XS[j, 2 * TB:, :] = X[:TB] + X[TB:]

            sg = 1.0 - 2.0 * (lax.broadcasted_iota(jnp.int32, (TB, CC), 0) & 1).astype(f32)
            prev = None
            cps[c][2].wait()
            for m in range(NB):
                K = lax.dot_general(fw, sb[c, :, m * TB:(m + 1) * TB],
                                    (((1,), (1,)), ((), ())), preferred_element_type=f32)
                kr, ki = K[:TB], K[TB:]
                if prev is not None:
                    kr = kr - sg * prev[TB:]
                    ki = ki + sg * prev[:TB]
                prev = K
                KS[m, 0:TB, :] = kr + ki
                KS[m, TB:2 * TB, :] = ki - kr
                KS[m, 2 * TB:, :] = kr

            def pos(p, _):
                for g in range(NB // 4):
                    for l in range(CC // 128):
                        spec(g, pl.multiple_of(p * 8, 8), l, 4 * g)
                return 0
            lax.fori_loop(0, TB // 8, pos, 0, unroll=PU)
            for g in range(NB // 4):
                inv(c, g, 4 * g)

    pl.run_scoped(conv, pltpu.VMEM((NC, S, CC), bf16), pltpu.VMEM((NC, S, CC), bf16),
                  pltpu.VMEM((NC, CC, S), bf16))

    def mixer(xa, xn, H, nb):
        G = D // 4
        ob = qb
        H[0:8, :] = jnp.zeros((8, D), f32)
        H[8 + S:, :] = jnp.zeros((8, D), f32)

        def rows(t, off=0, n=TM):
            r = t * TM + off
            return pl.ds(r if isinstance(r, int) else pl.multiple_of(r, 8), n)

        def pre(src, t, l):
            n2 = []
            for u in range(TM // RS):
                rs = rows(t, u * RS, RS)
                x = src[rs, :].astype(f32)
                x = x + _ln(x) * jnp.concatenate([yb[c, rs, :] for c in range(NC)], 1)
                c = x - jnp.mean(x, axis=-1, keepdims=True)
                v = jnp.mean(c * c, axis=-1, keepdims=True)
                r = lax.rsqrt(v + EPS)
                xa[rs, :] = x
                xn[rs, :] = c * r
                n2.append((c * (r * lax.rsqrt(v * r * r + EPS))).astype(bf16))
                yield
            H[rows(t, 8), :] = _gelu(_dot(jnp.concatenate(n2, 0), w1[...]))

        def mix(t, l):
            parts = []
            for g, sh in enumerate((1, -1, 2, -2)):
                w = H[rows(t, 0, TM + 16), g * G:(g + 1) * G]
                parts.append(pltpu.roll(w, sh % (TM + 16), 0)[8:8 + TM].astype(bf16))
                yield
            hs = _dot(jnp.concatenate(parts, 1), w2[...])
            yield
            for u in range(TM // RS):
                rs = rows(t, u * RS, RS)
                xu = xn[rs, :] + hs[u * RS:(u + 1) * RS]
                nb[t % 2, u * RS:(u + 1) * RS, :] = _ln(xu).astype(bf16)
                xa[rs, :] = xa[rs, :] + xu
                yield

        def mlp(t, l, first=False):
            n1 = nb[t % 2]
            acc = xa[rows(t), :]
            for fc in range(F // FC):
                if first and fc == F // FC // 2:
                    for cp in wcopies[5:]:
                        cp.wait()
                u = _dot(n1, w3[:, fc * FC:(fc + 1) * FC])
                g = _gelu(u).astype(bf16)
                yield
                d = _dot(g, w4[fc * FC:(fc + 1) * FC, :])
                acc = acc + d
                yield
            if l == 0:
                xa[rows(t), :] = acc
            else:
                ob[rows(t), :] = acc.astype(bf16)
                ocp(t).start()

        def ocp(t):
            return pltpu.make_async_copy(ob.at[rows(t)], out_h.at[rows(t)], sem_o.at[t])

        def chain(*gs):
            for g in gs:
                yield from g
                yield

        def weave(a, *bs):
            n = 0
            for _ in a:
                n += 1
                for i, b in enumerate(bs):
                    if i or n % SK == 0:
                        next(b, None)
            for b in bs:
                for _ in b:
                    pass

        wcopies[0].wait()
        wcopies[1].wait()

        def s0(t, _):
            weave(pre(qb, t, 0))
            return 0
        lax.fori_loop(0, 2, s0, 0)
        wcopies[2].wait()
        weave(mix(0, 0))
        wcopies[3].wait()
        wcopies[4].wait()
        weave(mlp(0, 0, True), chain(pre(qb, 2, 0), mix(1, 0)))

        def s1(t, _):
            weave(mlp(t, 0), chain(pre(qb, t + 2, 0), mix(t + 1, 0)))
            return 0
        lax.fori_loop(1, NT - 2, s1, 0)
        weave(mlp(NT - 2, 0), chain(pre(xa, 0, 1), mix(NT - 1, 0)))
        weave(mlp(NT - 1, 0), chain(pre(xa, 1, 1), mix(0, 1)))

        def s2(t, _):
            weave(mlp(t, 1), chain(pre(xa, t + 2, 1), mix(t + 1, 1)))
            return 0
        lax.fori_loop(0, NT - 2, s2, 0)
        weave(mlp(NT - 2, 1), mix(NT - 1, 1))
        weave(mlp(NT - 1, 1))
        for t in range(NT):
            ocp(t).wait()

    pl.run_scoped(mixer, pltpu.VMEM((S, D), f32), pltpu.VMEM((S, D), f32),
                  pltpu.VMEM((S + 16, D), f32), pltpu.VMEM((2, TM, D), bf16))


@jax.jit
def pallas_interleave_layers__ssm_conv_h3__mixer_s_mlp__prompt_kernel(
    A_q, A_k, A_v, A_shift_k, A_ssm_k, A_ssm_D, B_x, B_w1, B_w2, B_w3, B_w4,
):
    del B_x
    fw, iv = _dft_mats()
    hbm = pl.BlockSpec(memory_space=pl.ANY)
    vm = pl.BlockSpec(memory_space=pltpu.VMEM)
    out = pl.pallas_call(
        _kernel,
        out_shape=jax.ShapeDtypeStruct((S, D), bf16),
        in_specs=[hbm, hbm, hbm, vm, hbm, vm, hbm, hbm, hbm, hbm, vm, vm],
        out_specs=hbm,
        scratch_shapes=[
            pltpu.VMEM((S, D), bf16), pltpu.VMEM((D, D), bf16), pltpu.VMEM((D, D), bf16),
            pltpu.VMEM((D, F), bf16), pltpu.VMEM((F, D), bf16), pltpu.VMEM((NC, S, CC), f32),
            pltpu.VMEM((NB, 3 * TB, CC), f32), pltpu.VMEM((NB, 3 * TB, CC), f32),
            pltpu.VMEM((4, 4, 2 * TB, CC), f32),
            pltpu.SemaphoreType.DMA((3 * NC,)), pltpu.SemaphoreType.DMA((7,)),
            pltpu.SemaphoreType.DMA((NT,)),
        ],
        compiler_params=pltpu.CompilerParams(vmem_limit_bytes=112 * 1024 * 1024),
    )(A_q.reshape(S, D), A_k.reshape(S, D), A_v.reshape(S, D),
      A_shift_k.T.astype(f32), A_ssm_k, A_ssm_D.reshape(1, D).astype(f32),
      B_w1, B_w2, B_w3, B_w4, jnp.asarray(fw, bf16), jnp.asarray(iv, bf16))
    return out.reshape(1, S, D)
```

```python
import numpy as np
import jax
import jax.numpy as jnp
from jax import lax
import jax.experimental.pallas as pl
import jax.experimental.pallas.tpu as pltpu

S, D, F = 2048, 1024, 3584
TB = 128
NB = S // TB
CC = 256
NC = D // CC
TM = 256
NT = S // TM
FC = 256
RS = 256
EPS = 1e-5
SK = 3
f32, bf16 = jnp.float32, jnp.bfloat16


def _dft_mats():
    t = np.arange(TB)
    ang = 2 * np.pi * np.outer(t + 0.5, t) / (2 * TB)
    fwd = np.concatenate([np.cos(ang), -np.sin(ang)], 0)
    return fwd.astype(np.float32), (fwd.T / TB).astype(np.float32)


def _ln(x):
    m = jnp.mean(x, axis=-1, keepdims=True)
    c = x - m
    v = jnp.mean(c * c, axis=-1, keepdims=True)
    return c * lax.rsqrt(v + EPS)


def _gelu(x):
    c0 = float(np.sqrt(2 / np.pi))
    u = x * (x * x * (0.044715 * c0) + c0)
    hx = 0.5 * x
    return hx * jnp.tanh(u) + hx


def _dot(a, b):
    return jnp.dot(a, b, preferred_element_type=f32)


def _kernel(q_h, k_h, v_h, sk_ref, ssm_h, sd_ref, w1_h, w2_h, w3_h, w4_h,
            fw_ref, iv_ref, out_h,
            qb, w1, w2, w3, w4, yb, XS, KS, ZS, sem_in, sem_w, sem_o):
    FH = F // 2
    wcopies = [pltpu.make_async_copy(a, b, sem_w.at[i]) for i, (a, b) in enumerate((
        (q_h, qb), (w1_h, w1), (w2_h, w2),
        (w3_h.at[:, :FH], w3.at[:, :FH]), (w4_h.at[:FH], w4.at[:FH]),
        (w3_h.at[:, FH:], w3.at[:, FH:]), (w4_h.at[FH:], w4.at[FH:])))]

    def spec(zc, r, l, i0):
        ls = pl.ds(l * 128, 128)
        ld = lambda ref, b, comp: ref[b, pl.ds(r + comp * TB, 8), ls]
        acc = [[None] * 3 for _ in range(4)]
        for j in range(i0 + 4):
            a, b, ab = ld(XS, j, 0), ld(XS, j, 1), ld(XS, j, 2)
            for ii in range(4):
                m = i0 + ii - j
                if m >= 0:
                    t = (b * ld(KS, m, 0), a * ld(KS, m, 1), ab * ld(KS, m, 2))
                    acc[ii] = [u if o is None else o + u for o, u in zip(acc[ii], t)]
        for ii in range(4):
            ZS[zc, ii, pl.ds(r, 8), ls] = acc[ii][2] - acc[ii][0]
            ZS[zc, ii, pl.ds(r + TB, 8), ls] = acc[ii][2] + acc[ii][1]

    def inv(c, zc, i0):
        for ii in range(4):
            rs = pl.ds((i0 + ii) * TB, TB)
            yb[c, rs, :] = _dot(iv_ref[...], ZS[zc, ii].astype(bf16))

    def conv(kb, vb, sb):
        cps = []
        for c in range(NC):
            cs = pl.ds(c * CC, CC)
            cps.append([
                pltpu.make_async_copy(k_h.at[:, cs], kb.at[c], sem_in.at[3 * c]),
                pltpu.make_async_copy(v_h.at[:, cs], vb.at[c], sem_in.at[3 * c + 1]),
                pltpu.make_async_copy(ssm_h.at[cs, :], sb.at[c], sem_in.at[3 * c + 2]),
            ])
        later = [wcopies[:1], wcopies[1:3], wcopies[3:5], wcopies[5:]]
        for cp in cps[0]:
            cp.start()

        skt = sk_ref[...]
        sdf = sd_ref[...]

        for c in range(NC):
            cps[c][0].wait()
            if c + 1 < NC:
                for cp in cps[c + 1]:
                    cp.start()
            for cp in later[c]:
                cp.start()
            cps[c][1].wait()
            taps = [skt[j:j + 1, c * CC:(c + 1) * CC] for j in range(4)]
            sd = sdf[:, c * CC:(c + 1) * CC]
            fw = fw_ref[...]
            for j in range(NB):
                r0 = j * TB
                if j == 0:
                    kw = jnp.concatenate(
                        [jnp.zeros((16, CC), f32), kb[c, 0:TB, :].astype(f32)], 0)
                else:
                    kw = kb[c, r0 - 16:r0 + TB, :].astype(f32)
                kw = kw[8:]
                ks = kw[8:] * taps[0]
                for t in range(1, 4):
                    ks = ks + pltpu.roll(kw, t, 0)[8:] * taps[t]
                kv = ks * vb[c, r0:r0 + TB, :].astype(f32)
                X = _dot(fw, kv.astype(bf16))
                XS[j, :2 * TB, :] = X
                XS[j, 2 * TB:, :] = X[:TB] + X[TB:]

            sg = 1.0 - 2.0 * (lax.broadcasted_iota(jnp.int32, (TB, CC), 0) & 1).astype(f32)
            prev = None
            cps[c][2].wait()
            for m in range(NB):
                K = lax.dot_general(fw, sb[c, :, m * TB:(m + 1) * TB],
                                    (((1,), (1,)), ((), ())), preferred_element_type=f32)
                kr, ki = K[:TB], K[TB:]
                if m == 0:
                    kr = kr + sd
                cur = (kr, ki)
                if prev is not None:
                    kr = kr - sg * prev[1]
                    ki = ki + sg * prev[0]
                prev = cur
                KS[m, 0:TB, :] = kr + ki
                KS[m, TB:2 * TB, :] = ki - kr
                KS[m, 2 * TB:, :] = kr

            def pos(p, _):
                for g in range(NB // 4):
                    for l in range(CC // 128):
                        spec(g, pl.multiple_of(p * 8, 8), l, 4 * g)
                return 0
            lax.fori_loop(0, TB // 8, pos, 0)
            for g in range(NB // 4):
                inv(c, g, 4 * g)

    pl.run_scoped(conv, pltpu.VMEM((NC, S, CC), bf16), pltpu.VMEM((NC, S, CC), bf16),
                  pltpu.VMEM((NC, CC, S), bf16))

    def mixer(xa, xn, H, nb):
        G = D // 4
        ob = qb
        H[0:8, :] = jnp.zeros((8, D), f32)
        H[8 + S:, :] = jnp.zeros((8, D), f32)

        def rows(t, off=0, n=TM):
            r = t * TM + off
            return pl.ds(r if isinstance(r, int) else pl.multiple_of(r, 8), n)

        def pre(src, t, l):
            n2 = []
            for u in range(TM // RS):
                rs = rows(t, u * RS, RS)
                x = src[rs, :].astype(f32)
                x = x + _ln(x) * jnp.concatenate([yb[c, rs, :] for c in range(NC)], 1)
                c = x - jnp.mean(x, axis=-1, keepdims=True)
                v = jnp.mean(c * c, axis=-1, keepdims=True)
                r = lax.rsqrt(v + EPS)
                xa[rs, :] = x
                xn[rs, :] = c * r
                n2.append((c * (r * lax.rsqrt(v * r * r + EPS))).astype(bf16))
                yield
            H[rows(t, 8), :] = _gelu(_dot(jnp.concatenate(n2, 0), w1[...]))

        def mix(t, l):
            parts = []
            for g, sh in enumerate((1, -1, 2, -2)):
                w = H[rows(t, 0, TM + 16), g * G:(g + 1) * G]
                parts.append(pltpu.roll(w, sh % (TM + 16), 0)[8:8 + TM].astype(bf16))
                yield
            hs = _dot(jnp.concatenate(parts, 1), w2[...])
            yield
            for u in range(TM // RS):
                rs = rows(t, u * RS, RS)
                xu = xn[rs, :] + hs[u * RS:(u + 1) * RS]
                nb[t % 2, u * RS:(u + 1) * RS, :] = _ln(xu).astype(bf16)
                xa[rs, :] = xa[rs, :] + xu
                yield

        def mlp(t, l):
            n1 = nb[t % 2]
            acc = xa[rows(t), :]
            for fc in range(F // FC):
                u = _dot(n1, w3[:, fc * FC:(fc + 1) * FC])
                g = _gelu(u).astype(bf16)
                yield
                d = _dot(g, w4[fc * FC:(fc + 1) * FC, :])
                acc = acc + d
                yield
            if l == 0:
                xa[rows(t), :] = acc
            else:
                ob[rows(t), :] = acc.astype(bf16)
                ocp(t).start()

        def ocp(t):
            return pltpu.make_async_copy(ob.at[rows(t)], out_h.at[rows(t)], sem_o.at[t])

        def chain(*gs):
            for g in gs:
                yield from g
                yield

        def weave(a, *bs):
            n = 0
            for _ in a:
                n += 1
                for i, b in enumerate(bs):
                    if i or n % SK == 0:
                        next(b, None)
            for b in bs:
                for _ in b:
                    pass

        wcopies[0].wait()
        wcopies[1].wait()

        def s0(t, _):
            weave(pre(qb, t, 0))
            return 0
        lax.fori_loop(0, 2, s0, 0)
        wcopies[2].wait()
        weave(mix(0, 0))
        for cp in wcopies[3:]:
            cp.wait()
        weave(mlp(0, 0), chain(pre(qb, 2, 0), mix(1, 0)))

        def s1(t, _):
            weave(mlp(t, 0), chain(pre(qb, t + 2, 0), mix(t + 1, 0)))
            return 0
        lax.fori_loop(1, NT - 2, s1, 0)
        weave(mlp(NT - 2, 0), chain(pre(xa, 0, 1), mix(NT - 1, 0)))
        weave(mlp(NT - 1, 0), chain(pre(xa, 1, 1), mix(0, 1)))

        def s2(t, _):
            weave(mlp(t, 1), chain(pre(xa, t + 2, 1), mix(t + 1, 1)))
            return 0
        lax.fori_loop(0, NT - 2, s2, 0)
        weave(mlp(NT - 2, 1), mix(NT - 1, 1))
        weave(mlp(NT - 1, 1))
        for t in range(NT):
            ocp(t).wait()

    pl.run_scoped(mixer, pltpu.VMEM((S, D), f32), pltpu.VMEM((S, D), f32),
                  pltpu.VMEM((S + 16, D), f32), pltpu.VMEM((2, TM, D), bf16))


@jax.jit
def pallas_interleave_layers__ssm_conv_h3__mixer_s_mlp__prompt_kernel(
    A_q, A_k, A_v, A_shift_k, A_ssm_k, A_ssm_D, B_x, B_w1, B_w2, B_w3, B_w4,
):
    del B_x
    fw, iv = _dft_mats()
    hbm = pl.BlockSpec(memory_space=pl.ANY)
    vm = pl.BlockSpec(memory_space=pltpu.VMEM)
    out = pl.pallas_call(
        _kernel,
        out_shape=jax.ShapeDtypeStruct((S, D), bf16),
        in_specs=[hbm, hbm, hbm, vm, hbm, vm, hbm, hbm, hbm, hbm, vm, vm],
        out_specs=hbm,
        scratch_shapes=[
            pltpu.VMEM((S, D), bf16), pltpu.VMEM((D, D), bf16), pltpu.VMEM((D, D), bf16),
            pltpu.VMEM((D, F), bf16), pltpu.VMEM((F, D), bf16), pltpu.VMEM((NC, S, CC), f32),
            pltpu.VMEM((NB, 3 * TB, CC), f32), pltpu.VMEM((NB, 3 * TB, CC), f32),
            pltpu.VMEM((4, 4, 2 * TB, CC), f32),
            pltpu.SemaphoreType.DMA((3 * NC,)), pltpu.SemaphoreType.DMA((7,)),
            pltpu.SemaphoreType.DMA((NT,)),
        ],
        compiler_params=pltpu.CompilerParams(vmem_limit_bytes=112 * 1024 * 1024),
    )(A_q.reshape(S, D), A_k.reshape(S, D), A_v.reshape(S, D),
      A_shift_k.T.astype(f32), A_ssm_k,
      A_ssm_D.reshape(1, D).astype(f32),
      B_w1, B_w2, B_w3, B_w4, jnp.asarray(fw, bf16), jnp.asarray(iv, bf16))
    return out.reshape(1, S, D)
```
